```python
import os as _os
_os.environ.setdefault("JAX_PLATFORMS", "cpu")
import jax
import jax.numpy as jnp

def _softmax(x, axis=-1):
    return jax.nn.softmax(x, axis=axis)
def _gelu(x):
    return jax.nn.gelu(x, approximate=True)
def _silu(x):
    return jax.nn.silu(x)
def _sigmoid(x):
    return jax.nn.sigmoid(x)
def _layernorm(x, axis=-1, eps=1e-5):
    m = jnp.mean(x, axis=axis, keepdims=True)
    v = jnp.var(x, axis=axis, keepdims=True)
    return (x - m) / jnp.sqrt(v + eps)
def _scatter_add(tgt, idx, src, axis=0):
    return tgt.at[idx].add(src)
def _segment_sum(src, seg, n):
    return jax.ops.segment_sum(src, seg, n)
class _Rng:
    def __init__(self, key):
        self._k = key
    def _next(self):
        self._k, sub = jax.random.split(self._k)
        return sub
    def normal(self, shape):
        return jax.random.normal(self._next(), shape, dtype=jnp.bfloat16)
    def randint(self, lo, hi, shape):
        return jax.random.randint(self._next(), shape, lo, hi, dtype=jnp.int32)
    def uniform(self, shape, lo=0.0, hi=1.0):
        return jax.random.uniform(self._next(), shape, jnp.bfloat16, lo, hi)
    def permutation(self, n):
        return jax.random.permutation(self._next(), n)


kernel_name = 'gated_mix__sliding_block_cached__mha_block_cached__decode'

def setup_inputs():
    _rng = _Rng(jax.random.key(int.from_bytes(__import__("os").urandom(4), "little")))
    _w = (lambda a: (lambda t: t.astype(jnp.bfloat16) if jnp.issubdtype(t.dtype, jnp.floating) else t)(jnp.asarray(a)))
    def _A_setup():
        B, Sq, D = 2, 1, 640
        Hq, Hkv, Sk, Dh = 32, 32, 4096, 128
        assert Hq % Hkv == 0, (Hq, Hkv)
        return {
            "x": _w((lambda *s: _rng.normal(s) * 0.05)(B, Sq, D)),
            "k_cache": _w((lambda *s: _rng.normal(s) * 3.2)(B, Hkv, Sk, Dh)),
            "v_cache": _w((lambda *s: _rng.normal(s) * 0.05)(B, Hkv, Sk, Dh)),
            "wq": _w((lambda *s: _rng.normal(s) * 3.2)(D, Hq * Dh) * (D ** -0.5)),
            "wo": _w((lambda *s: _rng.normal(s) * 0.05)(Hq * Dh, D) * ((Hq * Dh) ** -0.5)),
        }
    _A_in = _A_setup()

    def _B_setup():
        B, Sq, D = 2, 1, 640
        H, Sk, Dh = 32, 4096, 128
        return {
            "x": _w((lambda *s: _rng.normal(s) * 0.05)(B, Sq, D)),
            "k_cache": _w((lambda *s: _rng.normal(s) * 3.2)(B, H, Sk, Dh)),
            "v_cache": _w((lambda *s: _rng.normal(s) * 0.05)(B, H, Sk, Dh)),
            "wq": _w((lambda *s: _rng.normal(s) * 3.2)(D, H * Dh) * (D ** -0.5)),
            "wo": _w((lambda *s: _rng.normal(s) * 0.05)(H * Dh, D) * ((H * Dh) ** -0.5)),
        }
    _B_in = _B_setup()

    return {
        "A_x": _A_in["x"],
        "A_k_cache": _A_in["k_cache"],
        "A_v_cache": _A_in["v_cache"],
        "A_wq": _A_in["wq"],
        "A_wo": _A_in["wo"],
        "B_x": _B_in["x"],
        "B_k_cache": _B_in["k_cache"],
        "B_v_cache": _B_in["v_cache"],
        "B_wq": _B_in["wq"],
        "B_wo": _B_in["wo"],
        "gate_w": _w((lambda *s: _rng.normal(s) * 0.05)(640) * 16.0),
    }

def reference(A_x, A_k_cache, A_v_cache, A_wq, A_wo, B_x, B_k_cache, B_v_cache, B_wq, B_wo, gate_w):
    def _A_ref(x, k_cache, v_cache, wq, wo):
        B, Sq, D = x.shape
        Hq, Dh = 32, 128
        Hkv, Sk = k_cache.shape[1], k_cache.shape[2]
        W = min(4096, max(256, Sk // 4))
        rep = Hq // Hkv
        q = (lambda x, *d: x.transpose(*d))((x @ wq).reshape(B, Sq, Hq, Dh), 0, 2, 1, 3)
        k = jnp.repeat(k_cache[:, :, Sk - W:, :], rep, axis=1)
        v = jnp.repeat(v_cache[:, :, Sk - W:, :], rep, axis=1)
        scores = jnp.einsum("bhqd,bhkd->bhqk", q, k) * (Dh ** -0.5)
        p = _softmax(scores, axis=-1)
        o = jnp.einsum("bhqk,bhkd->bhqd", p, v)
        return (lambda x, *d: x.transpose(*d))(o, 0, 2, 1, 3).reshape(B, Sq, Hq * Dh) @ wo

    def _B_ref(x, k_cache, v_cache, wq, wo):
        B, Sq, D = x.shape
        H, Dh = 32, 128
        q = (lambda x, *d: x.transpose(*d))((x @ wq).reshape(B, Sq, H, Dh), 0, 2, 1, 3)
        scores = jnp.einsum("bhqd,bhkd->bhqk", q, k_cache) * (Dh ** -0.5)
        p = _softmax(scores, axis=-1)
        o = jnp.einsum("bhqk,bhkd->bhqd", p, v_cache)
        return (lambda x, *d: x.transpose(*d))(o, 0, 2, 1, 3).reshape(B, Sq, H * Dh) @ wo

    x = A_x
    g = _sigmoid((x * gate_w).sum(-1, keepdims=True))
    a = _A_ref(x, A_k_cache, A_v_cache, A_wq, A_wo)
    b = _B_ref(x, B_k_cache, B_v_cache, B_wq, B_wo)
    return g * a + (1 - g) * b
```

```python
import functools

import jax
import jax.numpy as jnp
import numpy as np
from jax import lax
import jax.experimental.pallas as pl
import jax.experimental.pallas.tpu as pltpu

BF16 = jnp.bfloat16
F32 = jnp.float32


@jax.jit
def pallas_gated_mix__sliding_block_cached__mha_block_cached__decode_kernel(
    A_x: jax.Array,
    A_k_cache: jax.Array,
    A_v_cache: jax.Array,
    A_wq: jax.Array,
    A_wo: jax.Array,
    B_x: jax.Array,
    B_k_cache: jax.Array,
    B_v_cache: jax.Array,
    B_wq: jax.Array,
    B_wo: jax.Array,
    gate_w: jax.Array,
):
    del B_x
    B, H, SK, DH = B_k_cache.shape
    D = A_x.shape[-1]
    W = min(4096, max(256, SK // 4))
    TB, NS, seg = 256, 8, 64
    GH = 4
    NG = H // GH
    NA, NB = W // TB, SK // TB
    A_BLOCKS, B_BLOCKS = NG * NA, NG * NB
    N = A_BLOCKS + B_BLOCKS
    C = (DH ** -0.5) * float(np.log2(np.e))
    NWO = NS
    WO_R = 8
    WO_ROWS = (H * DH) // WO_R
    WO_STEP = WO_ROWS // NWO

    def kern(x_hbm, g_hbm, ak_hbm, av_hbm, aq_hbm, ao_hbm, bk_hbm, bv_hbm, bq_hbm, bo_hbm, o_ref,
             x_v, g_v, wq_v, wo_v, k_v, v_v, xl_v, gate_v, q_v, m_v, l_v, acc_v, lhs_v, sem_kv, sem_w, sem_o):

        def start_wq():
            def body(j, _):
                r = pl.multiple_of((j // 4) * 8, 8)
                c = pl.multiple_of((j % 4) * 1024, 1024)
                for i in range(5):
                    for t, src in ((1, bq_hbm), (0, aq_hbm)):
                        pltpu.make_async_copy(src.at[pl.ds(2 * i, 2), pl.ds(r, 8), pl.ds(c, 1024)],
                                              wq_v.at[t, pl.ds(2 * i, 2), pl.ds(r, 8), pl.ds(c, 1024)],
                                              sem_w.at[2]).start(priority=t)
                return None
            lax.fori_loop(0, 32, body, None)

        def start_kv(k_hbm, v_hbm, g, r0, slot):
            h0 = g * GH
            for j in range(TB // seg):
                r = pl.multiple_of(r0 + j * seg, seg)
                d = pl.ds(j * seg, seg)
                for b in range(B):
                    for i in range(GH // 2):
                        src = (b, pl.ds(h0 + 2 * i, 2), pl.ds(r, seg))
                        dst = (slot, b, pl.ds(2 * i, 2), d)
                        pltpu.make_async_copy(v_hbm.at[src], v_v.at[dst], sem_kv.at[1, slot]).start(priority=1)
                        pltpu.make_async_copy(k_hbm.at[src], k_v.at[dst], sem_kv.at[0, slot]).start(priority=0)

        def start_block(n, slot):
            @pl.when(n < A_BLOCKS)
            def _():
                start_kv(ak_hbm, av_hbm, n // NA, (SK - W) + (n % NA) * TB, slot)

            @pl.when(jnp.logical_and(n >= A_BLOCKS, n < N))
            def _():
                nb = n - A_BLOCKS
                start_kv(bk_hbm, bv_hbm, nb // NB, (nb % NB) * TB, slot)

            @pl.when(n >= N)
            def _():
                p = n - N
                for j in range(WO_STEP // 16):
                    r = pl.multiple_of(p * WO_STEP + j * 16, 16)
                    for i in range(WO_R // 2):
                        for t, src in ((1, bo_hbm), (0, ao_hbm)):
                            pltpu.make_async_copy(src.at[pl.ds(2 * i, 2), pl.ds(r, 16)],
                                                  wo_v.at[t, pl.ds(2 * i, 2), pl.ds(r, 16)],
                                                  sem_o.at[p]).start(priority=t)

        cx = pltpu.make_async_copy(x_hbm, x_v, sem_w.at[0])
        cg = pltpu.make_async_copy(g_hbm, g_v, sem_w.at[1])
        cx.start()
        cg.start()
        start_wq()
        lax.fori_loop(0, NS, lambda n, _: start_block(n, n), None)

        row = lax.broadcasted_iota(jnp.int32, (8, DH), 0)
        cx.wait()
        cg.wait()
        xf = x_v[...].astype(F32)
        rowd = lax.broadcasted_iota(jnp.int32, (8, D), 0)
        x8 = jnp.where(rowd < GH, xf[0:1], xf[1:2])
        xl_v[...] = x8.astype(BF16)
        gw = g_v[...].astype(F32)
        z = x8[:, 0:128] * gw[0:1]
        for c in range(1, D // 128):
            z = z + x8[:, c * 128:(c + 1) * 128] * gw[c:c + 1]
        gate = jax.nn.sigmoid(jnp.sum(z, axis=-1, keepdims=True))
        gate_v[0] = jnp.broadcast_to(gate, (8, DH))
        gate_v[1] = jnp.broadcast_to(1.0 - gate, (8, DH))
        pltpu.make_async_copy(wq_v, wq_v, sem_w.at[2]).wait()

        def block(n, _):
            slot = n % NS
            is_b = (n >= A_BLOCKS).astype(jnp.int32)
            nb = n - is_b * A_BLOCKS
            g = jnp.where(is_b == 1, nb // NB, nb // NA)
            j = jnp.where(is_b == 1, nb % NB, nb % NA)
            last = jnp.where(is_b == 1, NB - 1, NA - 1)

            @pl.when(j == 0)
            def _():
                c0 = pl.multiple_of(g * (GH * DH), GH * DH)
                r = None
                for kk in range(5):
                    w = wq_v[is_b, pl.ds(2 * kk, 2), :, pl.ds(c0, GH * DH)].reshape(128, GH * DH)
                    t = jnp.dot(xl_v[:, kk * 128:(kk + 1) * 128], w, preferred_element_type=F32)
                    r = t if r is None else r + t
                q = r[:, 0:DH]
                for i in range(1, GH):
                    q = jnp.where(row % GH == i, r[:, i * DH:(i + 1) * DH], q)
                q_v[...] = q.astype(BF16)
                m_v[...] = jnp.full((8, DH), -jnp.inf, F32)
                l_v[...] = jnp.zeros((8, DH), F32)
                acc_v[...] = jnp.zeros((8, DH), F32)

            pltpu.make_async_copy(k_v.at[slot], k_v.at[slot], sem_kv.at[0, slot]).wait()
            pltpu.make_async_copy(v_v.at[slot], v_v.at[slot], sem_kv.at[1, slot]).wait()
            q = q_v[...]
            s = None
            for i in range(8):
                t = lax.dot_general(q, k_v[slot, i // GH, i % GH], (((1,), (1,)), ((), ())), preferred_element_type=F32)
                s = t if s is None else jnp.where(lax.broadcasted_iota(jnp.int32, (8, TB), 0) == i, t, s)
            m_old = m_v[...]
            m_new = jnp.maximum(m_old, jnp.max(s, axis=-1, keepdims=True))
            alpha = jnp.exp2((m_old - m_new) * C)
            ps = [jnp.exp2((s[:, c * 128:(c + 1) * 128] - m_new) * C) for c in range(TB // 128)]
            l_v[...] = alpha * l_v[...] + functools.reduce(lambda a, b: a + b, ps)
            m_v[...] = m_new
            p = jnp.concatenate(ps, axis=-1).astype(BF16)
            o = None
            for i in range(8):
                t = jnp.dot(p, v_v[slot, i // GH, i % GH], preferred_element_type=F32)
                o = t if o is None else jnp.where(row == i, t, o)
            acc_v[...] = alpha * acc_v[...] + o

            @pl.when(j == last)
            def _():
                on = acc_v[...] * (gate_v[is_b] / jnp.sum(l_v[...], axis=-1, keepdims=True))
                parts = []
                for i in range(GH):
                    a = on if i == 0 else pltpu.roll(on, 8 - i, 0)
                    b = pltpu.roll(on, 8 - (GH + i - 1), 0)
                    parts.append(jnp.where(row == 0, a, b))
                lhs_v[is_b, g] = jnp.concatenate(parts, axis=-1).astype(BF16)

            start_block(n + NS, slot)
            return None

        lax.fori_loop(0, N, block, None)

        acc = jnp.zeros((8, D), F32)
        ppt = 128 // WO_STEP
        for p0 in range(0, NWO, ppt):
            for p in range(p0, p0 + ppt):
                piece = wo_v.at[:, :, pl.ds(p * WO_STEP, WO_STEP)]
                pltpu.make_async_copy(piece, piece, sem_o.at[p]).wait()
            r0 = p0 * WO_STEP
            for t in range(2):
                for g in range(WO_R):
                    acc = acc + jnp.dot(lhs_v[t, g, :, r0:r0 + 128], wo_v[t, g, r0:r0 + 128, :], preferred_element_type=F32)
        o_ref[...] = acc[0:2].astype(BF16)

    hbm = pl.BlockSpec(memory_space=pltpu.HBM)
    out = pl.pallas_call(
        kern,
        out_shape=jax.ShapeDtypeStruct((B, D), BF16),
        in_specs=[hbm] * 10,
        out_specs=pl.BlockSpec(memory_space=pltpu.VMEM),
        scratch_shapes=[
            pltpu.VMEM((B, D), BF16), pltpu.VMEM((D // 128, 128), BF16),
            pltpu.VMEM((2, 10, 64, H * DH), BF16), pltpu.VMEM((2, WO_R, WO_ROWS, D), BF16),
            pltpu.VMEM((NS, B, GH, TB, DH), BF16), pltpu.VMEM((NS, B, GH, TB, DH), BF16),
            pltpu.VMEM((8, D), BF16), pltpu.VMEM((2, 8, DH), F32), pltpu.VMEM((8, DH), BF16),
            pltpu.VMEM((8, DH), F32), pltpu.VMEM((8, DH), F32), pltpu.VMEM((8, DH), F32),
            pltpu.VMEM((2, NG, 8, GH * DH), BF16),
            pltpu.SemaphoreType.DMA((2, NS)), pltpu.SemaphoreType.DMA((3,)), pltpu.SemaphoreType.DMA((NWO,)),
        ],
        compiler_params=pltpu.CompilerParams(vmem_limit_bytes=100 * 2**20, disable_bounds_checks=True),
        name="gated_mix_decode",
    )(A_x.reshape(B, D), gate_w.reshape(D // 128, 128), A_k_cache, A_v_cache,
      A_wq.reshape(10, 64, H * DH), A_wo.reshape(WO_R, WO_ROWS, D),
      B_k_cache, B_v_cache, B_wq.reshape(10, 64, H * DH), B_wo.reshape(WO_R, WO_ROWS, D))
    return out.reshape(B, 1, D)
```

```python
import functools

import jax
import jax.numpy as jnp
import numpy as np
from jax import lax
import jax.experimental.pallas as pl
import jax.experimental.pallas.tpu as pltpu

BF16 = jnp.bfloat16
F32 = jnp.float32

LANES = 128
GH = 8
TB = 256
SEG = 64
NS = 8
WQ_REGIONS = 10
WQ_SEGS = 5
WQ_COLS = 512
WO_REGIONS = 4
LEAD = 24
WO_TAIL = (4, 2, 1, 1)
LAST_ROWS = 32


def _decode_kernel(x_hbm, gw_hbm, ak_hbm, av_hbm, aq_hbm, ao_hbm, bk_hbm, bv_hbm, bq_hbm, bo_hbm, o_ref,
                   x_v, gw_v, wq_v, wo_v, k_v, v_v, xl_v, gate_v, q_v, m_v, l_v, acc_v, lhs_v, col_v,
                   sem_kv, sem_w, sem_o, *, window):
    B, D = x_v.shape
    BH, SK, DH = bk_hbm.shape
    H = BH // B
    head_groups = H // GH
    a_per_group, b_per_group = window // TB, SK // TB
    a_blocks = (BH // GH) * a_per_group
    n_blocks = a_blocks + (BH // GH) * b_per_group
    wo_rows = wo_v.shape[2]
    n_pieces = H // 2
    exp2_scale = (DH ** -0.5) * float(np.log2(np.e))
    wq_hbm, wo_hbm = (aq_hbm, bq_hbm), (ao_hbm, bo_hbm)

    def aligned(i, m):
        return i if isinstance(i, int) else pl.multiple_of(i, m)

    copies_per_row = WQ_REGIONS // WQ_SEGS
    col_blocks = H * DH // WQ_COLS

    def start_wq(t, e, priority):
        j = e // copies_per_row
        idx = (pl.ds(WQ_SEGS * (e % copies_per_row), WQ_SEGS),
               pl.ds(aligned((j // col_blocks) * 8, 8), 8),
               pl.ds(aligned((j % col_blocks) * WQ_COLS, WQ_COLS), WQ_COLS))
        pltpu.make_async_copy(wq_hbm[t].at[idx], wq_v.at[(t,) + idx], sem_w.at[2]).start(priority=priority)

    def start_kv(k_hbm, v_hbm, group, key0, slot):
        for j in range(TB // SEG):
            keys = pl.ds(pl.multiple_of(key0 + j * SEG, SEG), SEG)
            for i in range(GH // 2):
                for t, hbm, buf in ((1, v_hbm, v_v), (0, k_hbm, k_v)):
                    pltpu.make_async_copy(hbm.at[pl.ds(group * GH + 2 * i, 2), keys],
                                          buf.at[slot, pl.ds(2 * i, 2), pl.ds(j * SEG, SEG)],
                                          sem_kv.at[t, slot]).start(priority=t)

    def piece(n):
        return 2 * (n % (WO_REGIONS // 2)), aligned((n // (WO_REGIONS // 2)) * LANES, LANES)

    def start_wo(n, j):
        region, row0 = piece(n)
        for t in (1, 0):
            if t == 1 and isinstance(n, int) and n == n_pieces - 1:
                lo = (j % 4) * 32
                idx = (region + j // 4, pl.ds(row0 + lo, 32))
                sem = n if j < 4 else n_pieces + lo // LAST_ROWS
            else:
                idx = (pl.ds(region, 2), pl.ds(aligned(row0 + j * 16, 16), 16))
                sem = n
            pltpu.make_async_copy(wo_hbm[t].at[idx], wo_v.at[(t,) + idx], sem_o.at[t, sem]).start(priority=t)

    def start_block(n, slot):
        @pl.when(n < a_blocks)
        def _():
            start_kv(ak_hbm, av_hbm, n // a_per_group, (SK - window) + (n % a_per_group) * TB, slot)

        @pl.when(jnp.logical_and(n >= a_blocks, n < n_blocks))
        def _():
            nb = n - a_blocks
            start_kv(bk_hbm, bv_hbm, nb // b_per_group, (nb % b_per_group) * TB, slot)

        @pl.when(n >= n_blocks)
        def _():
            per_step = 8 * (n_pieces // 2) // NS
            for u in range(per_step):
                e = (n - n_blocks) * per_step + u
                start_wo((e // 16) * 2 + u % 2, (e % 16) // 2)

    for e in range(LEAD):
        start_wq(e % 2, e // 2, 1)

    @pl.loop(0, (col_blocks * (wq_v.shape[2] // 8) * copies_per_row - LEAD // 2) // copies_per_row)
    def _(j):
        for u in range(copies_per_row):
            start_wq(1, LEAD // 2 + j * copies_per_row + u, 1)
            start_wq(0, LEAD // 2 + j * copies_per_row + u, 0)

    copy_x = pltpu.make_async_copy(x_hbm, x_v, sem_w.at[0])
    copy_gw = pltpu.make_async_copy(gw_hbm, gw_v, sem_w.at[1])
    copy_x.start(priority=1)
    copy_gw.start(priority=0)

    row = lax.broadcasted_iota(jnp.int32, (GH, DH), 0)

    @pl.loop(0, n_blocks + NS)
    def _(it):
        n = it - NS
        slot = it % NS

        @pl.when(n == 0)
        def _():
            copy_x.wait()
            copy_gw.wait()
            x = x_v[...].astype(F32)
            gw = gw_v[...].astype(F32)
            for b in range(B):
                xb = jnp.broadcast_to(x[b:b + 1], (GH, D))
                xl_v[b] = xb.astype(BF16)
                z = functools.reduce(jnp.add, [xb[:, c * LANES:(c + 1) * LANES] * gw[c:c + 1]
                                               for c in range(D // LANES)])
                gate = jax.nn.sigmoid(jnp.sum(z, axis=-1, keepdims=True))
                gate_v[0, b] = jnp.broadcast_to(gate, (GH, DH))
                gate_v[1, b] = jnp.broadcast_to(1.0 - gate, (GH, DH))
            lhs_v[...] = jnp.zeros(lhs_v.shape, F32)
            pltpu.make_async_copy(wq_v, wq_v, sem_w.at[2]).wait()

        @pl.when(n >= 0)
        def _():
            branch = (n >= a_blocks).astype(jnp.int32)
            nb = n - branch * a_blocks
            group = jnp.where(branch == 1, nb // b_per_group, nb // a_per_group)
            j = jnp.where(branch == 1, nb % b_per_group, nb % a_per_group)
            last = jnp.where(branch == 1, b_per_group - 1, a_per_group - 1)
            b = group // head_groups
            hg = group % head_groups

            @pl.when(j == 0)
            def _():
                cols = pl.ds(pl.multiple_of(hg * (GH * DH), GH * DH), GH * DH)
                w = wq_v[branch, :, :, cols].reshape(D, GH * DH)
                r = jnp.dot(xl_v[b], w, preferred_element_type=F32)
                q = r[:, 0:DH]
                for i in range(1, GH):
                    q = jnp.where(row == i, r[:, i * DH:(i + 1) * DH], q)
                q_v[...] = q.astype(BF16)
                m_v[...] = jnp.full((GH, DH), -jnp.inf, F32)
                l_v[...] = jnp.zeros((GH, DH), F32)
                acc_v[...] = jnp.zeros((GH, DH), F32)

            pltpu.make_async_copy(k_v.at[slot], k_v.at[slot], sem_kv.at[0, slot]).wait()
            pltpu.make_async_copy(v_v.at[slot], v_v.at[slot], sem_kv.at[1, slot]).wait()

            q = q_v[...]
            key_row = lax.broadcasted_iota(jnp.int32, (GH, TB), 0)
            s = None
            for i in range(GH):
                t = lax.dot_general(q, k_v[slot, i], (((1,), (1,)), ((), ())), preferred_element_type=F32)
                s = t if s is None else jnp.where(key_row == i, t, s)

            m_old = m_v[...]
            m_new = jnp.maximum(m_old, jnp.max(s, axis=-1, keepdims=True))
            alpha = jnp.exp2((m_old - m_new) * exp2_scale)
            p = [jnp.exp2((s[:, c * LANES:(c + 1) * LANES] - m_new) * exp2_scale) for c in range(TB // LANES)]
            m_v[...] = m_new
            l_v[...] = alpha * l_v[...] + functools.reduce(jnp.add, p)

            p = jnp.concatenate(p, axis=-1).astype(BF16)
            o = None
            for i in range(GH):
                t = jnp.dot(p, v_v[slot, i], preferred_element_type=F32)
                o = t if o is None else jnp.where(row == i, t, o)
            acc_v[...] = alpha * acc_v[...] + o

            @pl.when(j == last)
            def _():
                out = acc_v[...] * (gate_v[branch, b] / jnp.sum(l_v[...], axis=-1, keepdims=True))
                for i in range(GH):
                    lhs_v[branch, hg * GH + i, pl.ds(b, 1), :] = out[i:i + 1]

        start_block(it, slot)

    def wait_wo(idx, sem):
        pltpu.make_async_copy(wo_v.at[idx], wo_v.at[idx], sem_o.at[idx[0], sem]).wait()

    def project_rows(t, region, row0, acc):
        lhs = lhs_v[t, (region * wo_rows + row0) // DH].astype(BF16)
        return acc + jnp.dot(lhs, wo_v[t, region, pl.ds(row0, DH), :], preferred_element_type=F32)

    def project_piece(t, n, acc):
        region, row0 = piece(n)
        wait_wo((t, pl.ds(region, 2), pl.ds(row0, DH)), n)
        return project_rows(t, region + 1, row0, project_rows(t, region, row0, acc))

    last_region, last_row0 = piece(n_pieces - 1)
    last_lhs = lhs_v[1, ((last_region + 1) * wo_rows + last_row0) // DH]
    for b in range(B):
        col_v[b] = jnp.broadcast_to(last_lhs[b:b + 1], (DH, DH)).T

    half = n_pieces // 2
    order, first = [], half
    for size in WO_TAIL:
        order += [(first + w, j) for j in range(8) for w in range(size)]
        first += size

    acc = jnp.zeros((GH, D), F32)
    for n in range(half):
        for piece_copy in order[8 * n:8 * n + 8]:
            start_wo(*piece_copy)
        acc = project_piece(1, n, project_piece(0, n, acc))
    ahead = 3
    for n in range(half, half + ahead):
        acc = project_piece(0, n, acc)
    for n in range(half, n_pieces - 1):
        if n + ahead < n_pieces:
            acc = project_piece(0, n + ahead, acc)
        acc = project_piece(1, n, acc)
    wait_wo((1, last_region, pl.ds(last_row0, DH)), n_pieces - 1)
    acc = project_rows(1, last_region, last_row0, acc)

    out_row = lax.broadcasted_iota(jnp.int32, (GH, D), 0)
    partial = [jnp.where(out_row == b, acc, 0.0) for b in range(B)]
    for c in range(DH // LAST_ROWS):
        rows = pl.ds(last_row0 + c * LAST_ROWS, LAST_ROWS)
        wait_wo((1, last_region + 1, rows), n_pieces + c)
        w = wo_v[1, last_region + 1, rows, :].astype(F32)
        for k in range(LAST_ROWS // 8):
            for b in range(B):
                col = col_v[b, pl.ds(c * LAST_ROWS + 8 * k, 8), :]
                partial[b] = partial[b] + w[8 * k:8 * k + 8] * jnp.tile(col, (1, D // LANES))
    o_ref[...] = jnp.concatenate([jnp.sum(p, axis=0, keepdims=True) for p in partial], axis=0).astype(BF16)


@jax.jit
def pallas_gated_mix__sliding_block_cached__mha_block_cached__decode_kernel(
    A_x: jax.Array,
    A_k_cache: jax.Array,
    A_v_cache: jax.Array,
    A_wq: jax.Array,
    A_wo: jax.Array,
    B_x: jax.Array,
    B_k_cache: jax.Array,
    B_v_cache: jax.Array,
    B_wq: jax.Array,
    B_wo: jax.Array,
    gate_w: jax.Array,
):
    del B_x
    B, H, SK, DH = B_k_cache.shape
    D = A_x.shape[-1]
    assert A_k_cache.shape == B_k_cache.shape and A_x.shape == (B, 1, D)
    assert DH == LANES and sum(WO_TAIL) == H // 4
    window = min(4096, max(256, SK // 4))

    heads = lambda cache: cache.reshape(B * H, SK, DH)
    wq_shape = (WQ_REGIONS, D // WQ_REGIONS, H * DH)
    wo_shape = (WO_REGIONS, H * DH // WO_REGIONS, D)

    out = pl.pallas_call(
        functools.partial(_decode_kernel, window=window),
        out_shape=jax.ShapeDtypeStruct((B, D), BF16),
        in_specs=[pl.BlockSpec(memory_space=pltpu.HBM)] * 10,
        out_specs=pl.BlockSpec(memory_space=pltpu.VMEM),
        scratch_shapes=[
            pltpu.VMEM((B, D), BF16),
            pltpu.VMEM((D // LANES, LANES), BF16),
            pltpu.VMEM((2,) + wq_shape, BF16),
            pltpu.VMEM((2,) + wo_shape, BF16),
            pltpu.VMEM((NS, GH, TB, DH), BF16),
            pltpu.VMEM((NS, GH, TB, DH), BF16),
            pltpu.VMEM((B, GH, D), BF16),
            pltpu.VMEM((2, B, GH, DH), F32),
            pltpu.VMEM((GH, DH), BF16),
            pltpu.VMEM((GH, DH), F32),
            pltpu.VMEM((GH, DH), F32),
            pltpu.VMEM((GH, DH), F32),
            pltpu.VMEM((2, H, GH, DH), F32),
            pltpu.VMEM((B, DH, DH), F32),
            pltpu.SemaphoreType.DMA((2, NS)),
            pltpu.SemaphoreType.DMA((3,)),
            pltpu.SemaphoreType.DMA((2, H // 2 + DH // LAST_ROWS)),
        ],
        compiler_params=pltpu.CompilerParams(
            vmem_limit_bytes=64 * 2**20,
            disable_bounds_checks=True,
            disable_semaphore_checks=True,
        ),
        name="gated_mix_decode",
    )(
        A_x.reshape(B, D), gate_w.reshape(D // LANES, LANES),
        heads(A_k_cache), heads(A_v_cache), A_wq.reshape(wq_shape), A_wo.reshape(wo_shape),
        heads(B_k_cache), heads(B_v_cache), B_wq.reshape(wq_shape), B_wo.reshape(wo_shape),
    )
    return out.reshape(B, 1, D)
```

```python
import functools

import jax
import jax.numpy as jnp
import numpy as np
from jax import lax
import jax.experimental.pallas as pl
import jax.experimental.pallas.tpu as pltpu

BF16 = jnp.bfloat16
F32 = jnp.float32

LANES = 128
GH = 8
TB = 256
SEG = 64
NS = 8
WQ_REGIONS = 10
WQ_SEGS = 5
WQ_COLS = 512
WO_REGIONS = 4
LEAD = 24
WO_TAIL = (4, 2, 1, 1)
LAST_ROWS = 32


def _decode(x_hbm, gw_hbm, ak_hbm, av_hbm, aq_hbm, ao_hbm, bk_hbm, bv_hbm, bq_hbm, bo_hbm, o_ref,
            x_v, gw_v, wq_v, wo_v, k_v, v_v, xl_v, gate_v, q_v, m_v, l_v, acc_v, lhs_v, col_v,
            sem_kv, sem_w, sem_o, *, window):
    B, D = x_v.shape
    BH, SK, DH = bk_hbm.shape
    H = BH // B
    head_groups = H // GH
    a_per_group, b_per_group = window // TB, SK // TB
    a_blocks = (BH // GH) * a_per_group
    n_blocks = a_blocks + (BH // GH) * b_per_group
    wo_rows = wo_v.shape[2]
    n_pieces = H // 2
    exp2_scale = (DH ** -0.5) * float(np.log2(np.e))
    wq_hbm, wo_hbm = (aq_hbm, bq_hbm), (ao_hbm, bo_hbm)

    def aligned(i, m):
        return i if isinstance(i, int) else pl.multiple_of(i, m)

    copies_per_row = WQ_REGIONS // WQ_SEGS
    col_blocks = H * DH // WQ_COLS

    def start_wq(t, e, priority):
        j = e // copies_per_row
        idx = (pl.ds(WQ_SEGS * (e % copies_per_row), WQ_SEGS),
               pl.ds(aligned((j // col_blocks) * 8, 8), 8),
               pl.ds(aligned((j % col_blocks) * WQ_COLS, WQ_COLS), WQ_COLS))
        pltpu.make_async_copy(wq_hbm[t].at[idx], wq_v.at[(t,) + idx], sem_w.at[2]).start(priority=priority)

    def start_kv(k_hbm, v_hbm, group, key0, slot):
        for j in range(TB // SEG):
            keys = pl.ds(pl.multiple_of(key0 + j * SEG, SEG), SEG)
            for i in range(GH // 2):
                for t, hbm, buf in ((1, v_hbm, v_v), (0, k_hbm, k_v)):
                    pltpu.make_async_copy(hbm.at[pl.ds(group * GH + 2 * i, 2), keys],
                                          buf.at[slot, pl.ds(2 * i, 2), pl.ds(j * SEG, SEG)],
                                          sem_kv.at[t, slot]).start(priority=t)

    def piece(n):
        return 2 * (n % (WO_REGIONS // 2)), aligned((n // (WO_REGIONS // 2)) * LANES, LANES)

    def start_wo(n, j):
        region, row0 = piece(n)
        for t in (1, 0):
            if t == 1 and isinstance(n, int) and n == n_pieces - 1:
                lo = (j % 4) * 32
                idx = (region + j // 4, pl.ds(row0 + lo, 32))
                sem = n if j < 4 else n_pieces + lo // LAST_ROWS
            else:
                idx = (pl.ds(region, 2), pl.ds(aligned(row0 + j * 16, 16), 16))
                sem = n
            pltpu.make_async_copy(wo_hbm[t].at[idx], wo_v.at[(t,) + idx], sem_o.at[t, sem]).start(priority=t)

    def start_block(n, slot):
        @pl.when(n < a_blocks)
        def _():
            start_kv(ak_hbm, av_hbm, n // a_per_group, (SK - window) + (n % a_per_group) * TB, slot)

        @pl.when(jnp.logical_and(n >= a_blocks, n < n_blocks))
        def _():
            nb = n - a_blocks
            start_kv(bk_hbm, bv_hbm, nb // b_per_group, (nb % b_per_group) * TB, slot)

        @pl.when(n >= n_blocks)
        def _():
            per_step = 8 * (n_pieces // 2) // NS
            for u in range(per_step):
                e = (n - n_blocks) * per_step + u
                start_wo((e // 16) * 2 + u % 2, (e % 16) // 2)

    for e in range(LEAD):
        start_wq(e % 2, e // 2, 1)

    @pl.loop(0, (col_blocks * (wq_v.shape[2] // 8) * copies_per_row - LEAD // 2) // copies_per_row)
    def _(j):
        for u in range(copies_per_row):
            start_wq(1, LEAD // 2 + j * copies_per_row + u, 1)
            start_wq(0, LEAD // 2 + j * copies_per_row + u, 0)

    copy_x = pltpu.make_async_copy(x_hbm, x_v, sem_w.at[0])
    copy_gw = pltpu.make_async_copy(gw_hbm, gw_v, sem_w.at[1])
    copy_x.start(priority=1)
    copy_gw.start(priority=0)

    row = lax.broadcasted_iota(jnp.int32, (GH, DH), 0)

    @pl.loop(0, n_blocks + NS)
    def _(it):
        n = it - NS
        slot = it % NS

        @pl.when(n == 0)
        def _():
            copy_x.wait()
            copy_gw.wait()
            x = x_v[...].astype(F32)
            gw = gw_v[...].astype(F32)
            for b in range(B):
                xb = jnp.broadcast_to(x[b:b + 1], (GH, D))
                xl_v[b] = xb.astype(BF16)
                z = functools.reduce(jnp.add, [xb[:, c * LANES:(c + 1) * LANES] * gw[c:c + 1]
                                               for c in range(D // LANES)])
                gate = jax.nn.sigmoid(jnp.sum(z, axis=-1, keepdims=True))
                gate_v[0, b] = jnp.broadcast_to(gate, (GH, DH))
                gate_v[1, b] = jnp.broadcast_to(1.0 - gate, (GH, DH))
            lhs_v[...] = jnp.zeros(lhs_v.shape, F32)
            pltpu.make_async_copy(wq_v, wq_v, sem_w.at[2]).wait()

        @pl.when(n >= 0)
        def _():
            branch = (n >= a_blocks).astype(jnp.int32)
            nb = n - branch * a_blocks
            group = jnp.where(branch == 1, nb // b_per_group, nb // a_per_group)
            j = jnp.where(branch == 1, nb % b_per_group, nb % a_per_group)
            last = jnp.where(branch == 1, b_per_group - 1, a_per_group - 1)
            b = group // head_groups
            hg = group % head_groups

            @pl.when(j == 0)
            def _():
                cols = pl.ds(pl.multiple_of(hg * (GH * DH), GH * DH), GH * DH)
                w = wq_v[branch, :, :, cols].reshape(D, GH * DH)
                r = jnp.dot(xl_v[b], w, preferred_element_type=F32)
                q = r[:, 0:DH]
                for i in range(1, GH):
                    q = jnp.where(row == i, r[:, i * DH:(i + 1) * DH], q)
                q_v[...] = q.astype(BF16)
                m_v[...] = jnp.full((GH, DH), -jnp.inf, F32)
                l_v[...] = jnp.zeros((GH, DH), F32)
                acc_v[...] = jnp.zeros((GH, DH), F32)

            pltpu.make_async_copy(k_v.at[slot], k_v.at[slot], sem_kv.at[0, slot]).wait()
            pltpu.make_async_copy(v_v.at[slot], v_v.at[slot], sem_kv.at[1, slot]).wait()

            q = q_v[...]
            key_row = lax.broadcasted_iota(jnp.int32, (GH, TB), 0)
            s = None
            for i in range(GH):
                t = lax.dot_general(q, k_v[slot, i], (((1,), (1,)), ((), ())), preferred_element_type=F32)
                s = t if s is None else jnp.where(key_row == i, t, s)

            m_old = m_v[...]
            m_new = jnp.maximum(m_old, jnp.max(s, axis=-1, keepdims=True))
            alpha = jnp.exp2((m_old - m_new) * exp2_scale)
            p = [jnp.exp2((s[:, c * LANES:(c + 1) * LANES] - m_new) * exp2_scale) for c in range(TB // LANES)]
            m_v[...] = m_new
            l_v[...] = alpha * l_v[...] + functools.reduce(jnp.add, p)

            p = jnp.concatenate(p, axis=-1).astype(BF16)
            o = None
            for i in range(GH):
                t = jnp.dot(p, v_v[slot, i], preferred_element_type=F32)
                o = t if o is None else jnp.where(row == i, t, o)
            acc_v[...] = alpha * acc_v[...] + o

            @pl.when(j == last)
            def _():
                out = acc_v[...] * (gate_v[branch, b] / jnp.sum(l_v[...], axis=-1, keepdims=True))
                for i in range(GH):
                    lhs_v[branch, hg * GH + i, pl.ds(b, 1), :] = out[i:i + 1]

        start_block(it, slot)

    def wait_wo(idx, sem):
        pltpu.make_async_copy(wo_v.at[idx], wo_v.at[idx], sem_o.at[idx[0], sem]).wait()

    def project_rows(t, region, row0, acc):
        lhs = lhs_v[t, (region * wo_rows + row0) // DH].astype(BF16)
        return acc + jnp.dot(lhs, wo_v[t, region, pl.ds(row0, DH), :], preferred_element_type=F32)

    def project_piece(t, n, acc):
        region, row0 = piece(n)
        wait_wo((t, pl.ds(region, 2), pl.ds(row0, DH)), n)
        return project_rows(t, region + 1, row0, project_rows(t, region, row0, acc))

    last_region, last_row0 = piece(n_pieces - 1)
    last_lhs = lhs_v[1, ((last_region + 1) * wo_rows + last_row0) // DH]
    for b in range(B):
        col_v[b] = jnp.broadcast_to(last_lhs[b:b + 1], (DH, DH)).T

    half = n_pieces // 2
    order, first = [], half
    for size in WO_TAIL:
        order += [(first + w, j) for j in range(8) for w in range(size)]
        first += size

    acc = jnp.zeros((GH, D), F32)
    for n in range(half):
        for piece_copy in order[8 * n:8 * n + 8]:
            start_wo(*piece_copy)
        acc = project_piece(1, n, project_piece(0, n, acc))
    ahead = 3
    for n in range(half, half + ahead):
        acc = project_piece(0, n, acc)
    for n in range(half, n_pieces - 1):
        if n + ahead < n_pieces:
            acc = project_piece(0, n + ahead, acc)
        acc = project_piece(1, n, acc)
    wait_wo((1, last_region, pl.ds(last_row0, DH)), n_pieces - 1)
    acc = project_rows(1, last_region, last_row0, acc)

    out_row = lax.broadcasted_iota(jnp.int32, (GH, D), 0)
    partial = [jnp.where(out_row == b, acc, 0.0) for b in range(B)]
    for c in range(DH // LAST_ROWS):
        rows = pl.ds(last_row0 + c * LAST_ROWS, LAST_ROWS)
        wait_wo((1, last_region + 1, rows), n_pieces + c)
        w = wo_v[1, last_region + 1, rows, :].astype(F32)
        for k in range(LAST_ROWS // 8):
            for b in range(B):
                col = col_v[b, pl.ds(c * LAST_ROWS + 8 * k, 8), :]
                partial[b] = partial[b] + w[8 * k:8 * k + 8] * jnp.tile(col, (1, D // LANES))
    o_ref[...] = jnp.concatenate([jnp.sum(p, axis=0, keepdims=True) for p in partial], axis=0).astype(BF16)


@jax.jit
def pallas_gated_mix__sliding_block_cached__mha_block_cached__decode_kernel(
    A_x: jax.Array,
    A_k_cache: jax.Array,
    A_v_cache: jax.Array,
    A_wq: jax.Array,
    A_wo: jax.Array,
    B_x: jax.Array,
    B_k_cache: jax.Array,
    B_v_cache: jax.Array,
    B_wq: jax.Array,
    B_wo: jax.Array,
    gate_w: jax.Array,
):
    del B_x
    B, H, SK, DH = B_k_cache.shape
    D = A_x.shape[-1]
    assert A_k_cache.shape == B_k_cache.shape and A_x.shape == (B, 1, D)
    assert DH == LANES and sum(WO_TAIL) == H // 4
    window = min(4096, max(256, SK // 4))

    heads = lambda cache: cache.reshape(B * H, SK, DH)
    wq_shape = (WQ_REGIONS, D // WQ_REGIONS, H * DH)
    wo_shape = (WO_REGIONS, H * DH // WO_REGIONS, D)

    def kernel(*refs):
        pl.run_scoped(
            functools.partial(_decode, *refs, window=window),
            pltpu.SemaphoreType.DMA((2, NS)),
            pltpu.SemaphoreType.DMA((3,)),
            pltpu.SemaphoreType.DMA((2, H // 2 + DH // LAST_ROWS)),
        )

    out = pl.pallas_call(
        kernel,
        out_shape=jax.ShapeDtypeStruct((B, D), BF16),
        in_specs=[pl.BlockSpec(memory_space=pltpu.HBM)] * 10,
        out_specs=pl.BlockSpec(memory_space=pltpu.VMEM),
        scratch_shapes=[
            pltpu.VMEM((B, D), BF16),
            pltpu.VMEM((D // LANES, LANES), BF16),
            pltpu.VMEM((2,) + wq_shape, BF16),
            pltpu.VMEM((2,) + wo_shape, BF16),
            pltpu.VMEM((NS, GH, TB, DH), BF16),
            pltpu.VMEM((NS, GH, TB, DH), BF16),
            pltpu.VMEM((B, GH, D), BF16),
            pltpu.VMEM((2, B, GH, DH), F32),
            pltpu.VMEM((GH, DH), BF16),
            pltpu.VMEM((GH, DH), F32),
            pltpu.VMEM((GH, DH), F32),
            pltpu.VMEM((GH, DH), F32),
            pltpu.VMEM((2, H, GH, DH), F32),
            pltpu.VMEM((B, DH, DH), F32),
        ],
        compiler_params=pltpu.CompilerParams(vmem_limit_bytes=64 * 2**20),
        name="gated_mix_decode",
    )(
        A_x.reshape(B, D), gate_w.reshape(D // LANES, LANES),
        heads(A_k_cache), heads(A_v_cache), A_wq.reshape(wq_shape), A_wo.reshape(wo_shape),
        heads(B_k_cache), heads(B_v_cache), B_wq.reshape(wq_shape), B_wo.reshape(wo_shape),
    )
    return out.reshape(B, 1, D)
```
